```python
import os as _os
_os.environ.setdefault("JAX_PLATFORMS", "cpu")
import jax
import jax.numpy as jnp

def _softmax(x, axis=-1):
    return jax.nn.softmax(x, axis=axis)
def _gelu(x):
    return jax.nn.gelu(x, approximate=True)
def _silu(x):
    return jax.nn.silu(x)
def _sigmoid(x):
    return jax.nn.sigmoid(x)
def _layernorm(x, axis=-1, eps=1e-5):
    m = jnp.mean(x, axis=axis, keepdims=True)
    v = jnp.var(x, axis=axis, keepdims=True)
    return (x - m) / jnp.sqrt(v + eps)
def _scatter_add(tgt, idx, src, axis=0):
    return tgt.at[idx].add(src)
def _segment_sum(src, seg, n):
    return jax.ops.segment_sum(src, seg, n)
class _Rng:
    def __init__(self, key):
        self._k = key
    def _next(self):
        self._k, sub = jax.random.split(self._k)
        return sub
    def normal(self, shape):
        return jax.random.normal(self._next(), shape, dtype=jnp.bfloat16)
    def randint(self, lo, hi, shape):
        return jax.random.randint(self._next(), shape, lo, hi, dtype=jnp.int32)
    def uniform(self, shape, lo=0.0, hi=1.0):
        return jax.random.uniform(self._next(), shape, jnp.bfloat16, lo, hi)
    def permutation(self, n):
        return jax.random.permutation(self._next(), n)


kernel_name = 'concat_heads__sliding_local_dilated__sliding_block__prompt'

def setup_inputs():
    _rng = _Rng(jax.random.key(int.from_bytes(__import__("os").urandom(4), "little")))
    _w = (lambda a: (lambda t: t.astype(jnp.bfloat16) if jnp.issubdtype(t.dtype, jnp.floating) else t)(jnp.asarray(a)))
    def _A_setup():
        B, S, D = 1, 2048, 1024
        return {
            "x": _w((lambda *s: _rng.normal(s) * 0.2)(B, S, D)),
            "wqkv": _w((lambda *s: _rng.normal(s) * 0.2)(D, 3 * D)),
            "wo": _w((lambda *s: _rng.normal(s) * 0.05)(D, D)),
        }
    _A_in = _A_setup()

    def _B_setup():
        B, S, D = 1, 2048, 1024
        return {
            "x": _w((lambda *s: _rng.normal(s) * 0.2)(B, S, D)),
            "wqkv": _w((lambda *s: _rng.normal(s) * 0.2)(D, 3 * D)),
            "wo": _w((lambda *s: _rng.normal(s) * 0.05)(D, D)),
        }
    _B_in = _B_setup()

    return {
        "A_x": _A_in["x"],
        "A_wqkv": _A_in["wqkv"],
        "A_wo": _A_in["wo"],
        "B_x": _B_in["x"],
        "B_wqkv": _B_in["wqkv"],
        "B_wo": _B_in["wo"],
    }

def reference(A_x, A_wqkv, A_wo, B_x, B_wqkv, B_wo):
    def _A_ref(x, wqkv, wo):
        B, S, D = x.shape
        H = 32; Dh = D // H
        W, dil = 8, 2
        qkv = (lambda x, *d: x.transpose(*d))((x @ wqkv).reshape(B, S, 3, H, Dh), 2, 0, 3, 1, 4)
        q, k, v = qkv[0], qkv[1], qkv[2]
        scale = Dh ** -0.5
        pos = jnp.arange(S)
        off = jnp.arange(W) * dil
        idx = pos[:, None] - off[None, :]
        mask = idx >= 0
        idx_c = jnp.where(mask, idx, 0).reshape(-1)
        kg = k[:, :, idx_c, :].reshape(B, H, S, W, Dh)
        vg = v[:, :, idx_c, :].reshape(B, H, S, W, Dh)
        logits = jnp.einsum("bhsd,bhswd->bhsw", q, kg) * scale
        logits = jnp.where(mask[None, None, :, :], logits, -1e9)
        attn = _softmax(logits, axis=-1)
        o = jnp.einsum("bhsw,bhswd->bhsd", attn, vg)
        return (lambda x, *d: x.transpose(*d))(o, 0, 2, 1, 3).reshape(B, S, D) @ wo

    def _B_ref(x, wqkv, wo):
        B, S, D = x.shape
        H = 32; Dh = D // H; W = 256
        qkv = (lambda x, *d: x.transpose(*d))((x @ wqkv).reshape(B, S, 3, H, Dh), 2, 0, 3, 1, 4)
        q, k, v = qkv[0], qkv[1], qkv[2]
        scores = jnp.einsum("bhqd,bhkd->bhqk", q, k) * (Dh ** -0.5)
        idx = jnp.arange(S)
        mask = (idx[:, None] - idx[None, :] >= 0) & (idx[:, None] - idx[None, :] < W)
        scores = jnp.where(mask[None, None], scores, -1e9)
        p = _softmax(scores, axis=-1)
        o = jnp.einsum("bhqk,bhkd->bhqd", p, v)
        return (lambda x, *d: x.transpose(*d))(o, 0, 2, 1, 3).reshape(B, S, D) @ wo

    a = _A_ref(A_x, A_wqkv, A_wo)
    b = _B_ref(B_x, B_wqkv, B_wo)
    return jnp.concatenate([a, b], axis=-1)
```

```python
import functools

import jax
import jax.numpy as jnp
import numpy as np
from jax import lax
from jax.experimental import pallas as pl
from jax.experimental.pallas import tpu as pltpu

S, D, H, DH = 2048, 1024, 32, 32
T = 256
NT = T // 128
NEG = -1e30
BF = jnp.bfloat16
F32 = jnp.float32
QSCALE = float(DH ** -0.5 * np.log2(np.e))

CFG = dict(
    per_head_dot=False,
    proj_chunk=512,
)

_NT_DIMS = (((1,), (1,)), ((), ()))
_TN_DIMS = (((0,), (0,)), ((), ()))


def _dot(a, b):
    return jnp.dot(a, b, preferred_element_type=F32)


def _dot_nt(a, b):
    return lax.dot_general(a, b, _NT_DIMS, preferred_element_type=F32)


def _stack_q(qt):
    lane_head = lax.broadcasted_iota(jnp.int32, qt.shape, 1) // DH
    zero = jnp.zeros_like(qt)
    return jnp.concatenate([jnp.where(lane_head == h, qt, zero) for h in range(4)], axis=0)


def _kernel(xa_ref, wa_ref, woa_ref, xb_ref, wb_ref, wob_ref, o_ref,
            qa_ref, ka_ref, vta_ref, ota_ref, qb_ref, kb_ref, vtb_ref, otb_ref):
    i = pl.program_id(0)
    cur = i % 2
    prv = 1 - cur
    cfg = CFG

    def project(x_ref, w_ref, q_ref, k_ref, vt_ref):
        x = x_ref[...]
        C = cfg["proj_chunk"]
        for c in range(0, D, C):
            q = _dot(x, w_ref[:, c:c + C])
            q_ref[:, c:c + C] = (q * QSCALE).astype(BF)
            k = _dot(x, w_ref[:, D + c:D + c + C])
            k_ref[cur, :, c:c + C] = k.astype(BF)
            v = _dot(x, w_ref[:, 2 * D + c:2 * D + c + C])
            vt_ref[cur, c:c + C, :] = v.astype(BF).T

    @pl.when(i == 0)
    def _():
        ka_ref[1, T - 16:T, :] = jnp.zeros((16, D), BF)
        vta_ref[1, :, T - 128:T] = jnp.zeros((D, 128), BF)

    project(xa_ref, wa_ref, qa_ref, ka_ref, vta_ref)
    project(xb_ref, wb_ref, qb_ref, kb_ref, vtb_ref)

    row = lax.broadcasted_iota(jnp.int32, (128, 128), 0)
    col = lax.broadcasted_iota(jnp.int32, (128, 128), 1)
    upper = row > col
    rowa = lax.broadcasted_iota(jnp.int32, (144, 128), 0)
    cola = lax.broadcasted_iota(jnp.int32, (144, 128), 1)
    dist = cola + 16 - rowa
    band = (dist >= 0) & (dist <= 14) & ((dist & 1) == 0)

    def attn_a():
        for t in range(NT):
            q0 = i * T + t * 128
            mask = band & (rowa + (q0 - 16) >= 0)
            for g in range(D // 128):
                ls = slice(128 * g, 128 * g + 128)
                qs = _stack_q(qa_ref[128 * t:128 * t + 128, ls])
                if t == 0:
                    kp = ka_ref[prv, T - 16:T, ls]
                else:
                    kp = ka_ref[cur, 128 * t - 16:128 * t, ls]
                k = jnp.concatenate([kp, ka_ref[cur, 128 * t:128 * t + 128, ls]], axis=0)
                if not cfg["per_head_dot"]:
                    st = _dot_nt(k, qs)
                for h in range(4):
                    if cfg["per_head_dot"]:
                        s = _dot_nt(k, qs[128 * h:128 * h + 128])
                    else:
                        s = st[:, 128 * h:128 * h + 128]
                    s = jnp.where(mask, s, NEG)
                    m = jnp.max(s, axis=0, keepdims=True)
                    p = jnp.exp2(s - m)
                    l = jnp.sum(p, axis=0, keepdims=True)
                    pb = p.astype(BF)
                    pt = jnp.concatenate([jnp.zeros((112, 128), BF), pb], axis=0)
                    fs = slice(128 * g + 32 * h, 128 * g + 32 * h + 32)
                    if t == 0:
                        vp = vta_ref[prv, fs, T - 128:T]
                    else:
                        vp = vta_ref[cur, fs, 128 * t - 128:128 * t]
                    vt = jnp.concatenate([vp, vta_ref[cur, fs, 128 * t:128 * t + 128]], axis=1)
                    o = _dot(vt, pt)
                    ota_ref[fs, 128 * t:128 * t + 128] = (o * (1.0 / l)).astype(BF)

    def attn_b(first):
        for t in range(NT):
            tiles = [(prv, 0), (prv, 128), (cur, 0)] if t == 0 else [(prv, 128), (cur, 0), (cur, 128)]
            nvalid = (t + 1) if first else 3
            tiles = tiles[3 - nvalid:]
            for g in range(D // 128):
                ls = slice(128 * g, 128 * g + 128)
                qs = _stack_q(qb_ref[128 * t:128 * t + 128, ls])
                k = jnp.concatenate([kb_ref[sl, r:r + 128, ls] for sl, r in tiles], axis=0)
                if not cfg["per_head_dot"]:
                    st = _dot_nt(k, qs)
                for h in range(4):
                    if cfg["per_head_dot"]:
                        s = _dot_nt(k, qs[128 * h:128 * h + 128])
                    else:
                        s = st[:, 128 * h:128 * h + 128]
                    s_last = s[-128:]
                    if nvalid == 3:
                        c = jnp.where(upper, s[0:128], s_last)
                        s2 = jnp.concatenate([c, s[128:256]], axis=0)
                    elif nvalid == 2:
                        c = jnp.where(upper, NEG, s_last)
                        s2 = jnp.concatenate([c, s[0:128]], axis=0)
                    else:
                        s2 = jnp.where(upper, NEG, s_last)
                    m = jnp.max(s2, axis=0, keepdims=True)
                    p = jnp.exp2(s2 - m)
                    l = jnp.sum(p, axis=0, keepdims=True)
                    pc = p[0:128]
                    if nvalid == 3:
                        pt = jnp.concatenate([
                            jnp.where(upper, pc, 0.0).astype(BF),
                            p[128:256].astype(BF),
                            jnp.where(upper, 0.0, pc).astype(BF)], axis=0)
                    elif nvalid == 2:
                        pt = jnp.concatenate([p[128:256].astype(BF), pc.astype(BF)], axis=0)
                    else:
                        pt = pc.astype(BF)
                    fs = slice(128 * g + 32 * h, 128 * g + 32 * h + 32)
                    vt = jnp.concatenate([vtb_ref[sl, fs, r:r + 128] for sl, r in tiles], axis=1)
                    o = _dot(vt, pt)
                    otb_ref[fs, 128 * t:128 * t + 128] = (o * (1.0 / l)).astype(BF)

    attn_a()
    o_ref[:, 0:D] = lax.dot_general(ota_ref[...], woa_ref[...], _TN_DIMS,
                                    preferred_element_type=F32).astype(BF)

    @pl.when(i == 0)
    def _():
        attn_b(True)

    @pl.when(i > 0)
    def _():
        attn_b(False)

    o_ref[:, D:2 * D] = lax.dot_general(otb_ref[...], wob_ref[...], _TN_DIMS,
                                        preferred_element_type=F32).astype(BF)


@jax.jit
def pallas_concat_heads__sliding_local_dilated__sliding_block__prompt_kernel(
    A_x, A_wqkv, A_wo, B_x, B_wqkv, B_wo,
):
    xa = A_x.reshape(S, D)
    xb = B_x.reshape(S, D)

    def full(shape):
        return pl.BlockSpec(shape, lambda i: (0, 0), pipeline_mode=pl.Buffered(1))

    xspec = pl.BlockSpec((T, D), lambda i: (i, 0))
    out = pl.pallas_call(
        _kernel,
        grid=(S // T,),
        in_specs=[xspec, full((D, 3 * D)), full((D, D)), xspec, full((D, 3 * D)), full((D, D))],
        out_specs=pl.BlockSpec((T, 2 * D), lambda i: (i, 0)),
        out_shape=jax.ShapeDtypeStruct((S, 2 * D), BF),
        scratch_shapes=[
            pltpu.VMEM((T, D), BF), pltpu.VMEM((2, T, D), BF), pltpu.VMEM((2, D, T), BF), pltpu.VMEM((D, T), BF),
            pltpu.VMEM((T, D), BF), pltpu.VMEM((2, T, D), BF), pltpu.VMEM((2, D, T), BF), pltpu.VMEM((D, T), BF),
        ],
        compiler_params=pltpu.CompilerParams(
            dimension_semantics=("arbitrary",),
            vmem_limit_bytes=100 * 1024 * 1024,
        ),
        name="fused_attn",
    )(xa, A_wqkv, A_wo, xb, B_wqkv, B_wo)
    return out.reshape(1, S, 2 * D)
```

```python
import jax
import jax.numpy as jnp
import numpy as np
from jax import lax
from jax.experimental import pallas as pl
from jax.experimental.pallas import tpu as pltpu

S, D, H, DH = 2048, 1024, 32, 32
T = 256
NT = T // 128
NEG = -1e30
BF = jnp.bfloat16
F32 = jnp.float32
U32 = jnp.uint32
QSCALE = float(DH ** -0.5 * np.log2(np.e))

CFG = dict(
    skew_a=10,
    skew_b=10,
    pchunk=512,
    pa_chunk=512,
    pb_chunk=128,
    ochunk=128,
    obchunk=512,
    inflight=3,
    fill_a=True,
    fill_b=True,
    tail_keep=2,
    a_group_qk=False,
    resched=True,
    x1pos=1, xb0pos=1,
    chain=True,
)

_NT_DIMS = (((1,), (1,)), ((), ()))
_TN_DIMS = (((0,), (0,)), ((), ()))


def _dot(a, b):
    return jnp.dot(a, b, preferred_element_type=F32)


def _dot_nt(a, b):
    return lax.dot_general(a, b, _NT_DIMS, preferred_element_type=F32)


def _kernel(xa_hbm, wa_hbm, woa_hbm, xb_hbm, wb_hbm, wob_hbm, o_hbm,
            xa_buf, xb_buf, oa_buf, ob_buf, wa_ref, wb_ref, woa_ref, wob_ref,
            qa_ref, ka_ref, vta_ref, ota_ref, qb_ref, kb_ref, vtb_ref, otb_ref,
            sems, xsems, osems):
    i = pl.program_id(0)
    nsteps = pl.num_programs(0)
    cfg = CFG
    PC = cfg["pchunk"]

    wcopies = []
    for w_hbm, w_ref in ((wa_hbm, wa_ref), (wb_hbm, wb_ref)):
        for c in range(0, D, PC):
            for part in range(3):
                c0 = part * D + c
                wcopies.append((w_hbm.at[:, c0:c0 + PC], w_ref.at[:, c0:c0 + PC]))
    n_qkv = len(wcopies) // 2
    wcopies.append((woa_hbm, woa_ref))
    wcopies.append((wob_hbm, wob_ref))
    widx = {}
    n = 0
    for br in range(2):
        for c in range(0, D, PC):
            for part in range(3):
                widx[(br, part, c)] = n
                n += 1
    widx["woa"] = n
    widx["wob"] = n + 1

    def wcopy(j):
        src, dst = wcopies[j]
        return pltpu.make_async_copy(src, dst, sems.at[j])

    first = i == 0
    last = i == nsteps - 1
    cur = i % 2
    prv = 1 - cur
    bias = jnp.where(first, jnp.float32(NEG), jnp.float32(0.0))
    def xcopy(br, step, slot):
        src = (xa_hbm, xb_hbm)[br].at[pl.ds(pl.multiple_of(step * T, T), T), :]
        return pltpu.make_async_copy(src, (xa_buf, xb_buf)[br].at[slot], xsems.at[br, slot])

    OB = cfg["obchunk"]
    n_ob = D // OB

    def ocopy(piece, step, slot):
        rows = pl.ds(pl.multiple_of(step * T, T), T)
        if piece == 0:
            return pltpu.make_async_copy(oa_buf.at[slot], o_hbm.at[rows, 0:D], osems.at[slot, 0])
        c0 = (piece - 1) * OB
        return pltpu.make_async_copy(ob_buf.at[slot, :, c0:c0 + OB],
                                     o_hbm.at[rows, D + c0:D + c0 + OB], osems.at[slot, piece])

    queue = [("x", 0)] + [("w", j) for j in range(len(wcopies))]
    queue.insert(cfg["xb0pos"], ("x", 1))
    queue.insert(len(queue) - cfg["x1pos"], ("x1", 0))
    q_started = [0]
    q_done = [0]

    def q_start_upto(n):
        lo, hi = q_started[0], min(n, len(queue))
        if hi > lo:
            @pl.when(first)
            def _():
                for kind, j in queue[lo:hi]:
                    if kind == "x1":
                        @pl.when(jnp.logical_not(last))
                        def _():
                            xcopy(0, 1, 1).start()
                            xcopy(1, 1, 1).start()
                    else:
                        (xcopy(j, 0, 0) if kind == "x" else wcopy(j)).start()
            q_started[0] = hi

    def q_need(item):
        p = queue.index(item)
        while q_done[0] <= p:
            kind, j = queue[q_done[0]]
            if kind == "x":
                xcopy(j, i, cur).wait()
            elif kind == "w":
                @pl.when(first)
                def _(j=j):
                    wcopy(j).wait()
            q_done[0] += 1
            q_start_upto(q_done[0] + cfg["inflight"])

    def need(key):
        q_need(("w", widx[key]))

    def need_x(br):
        q_need(("x", br))

    def prefetch_x():
        @pl.when(jnp.logical_and(jnp.logical_not(first), jnp.logical_not(last)))
        def _():
            xcopy(0, i + 1, prv).start()
            xcopy(1, i + 1, prv).start()

    o_waited = set()

    def need_obuf(br):
        if br not in o_waited:
            o_waited.add(br)

            @pl.when(i >= 2)
            def _():
                for piece in ([0] if br == 0 else range(1, 1 + n_ob)):
                    ocopy(piece, i - 2, cur).wait()

    q_start_upto(cfg["inflight"])
    prefetch_x()

    @pl.when(first)
    def _():
        kb_ref[1] = jnp.zeros(kb_ref.shape[1:], U32)
        vtb_ref[1] = jnp.zeros(vtb_ref.shape[1:], U32)
        ka_ref[1, T // 2 - 8:T // 2, :] = jnp.zeros((8, D), U32)
        vta_ref[1, :, T - 128:T] = jnp.zeros((D // 2, 128), U32)

    def step():
        def proj(br, part, c, cw):
            x_ref, w_ref, q_ref, k_ref, vt_ref = (
                (xa_buf.at[cur], wa_ref, qa_ref, ka_ref, vta_ref) if br == 0
                else (xb_buf.at[cur], wb_ref, qb_ref, kb_ref, vtb_ref))
            need_x(br)
            for cc in range(c // PC * PC, c + cw, PC):
                need((br, part, cc))
            r = _dot(x_ref[...], w_ref[:, part * D + c:part * D + c + cw])
            if part == 0:
                q_ref[:, c:c + cw] = pltpu.bitcast((r * QSCALE).astype(BF), U32)
            elif part == 1:
                k_ref[cur, :, c:c + cw] = pltpu.bitcast(r.astype(BF), U32)
            else:
                vt_ref[cur, c // 2:(c + cw) // 2, :] = pltpu.bitcast(r.astype(BF).T, U32)

        row = lax.broadcasted_iota(jnp.int32, (128, 128), 0)
        col = lax.broadcasted_iota(jnp.int32, (128, 128), 1)
        upper = row > col
        lane_head = lax.broadcasted_iota(jnp.int32, (64, 128), 1) // DH

        def band(nrows):
            r = lax.broadcasted_iota(jnp.int32, (nrows, 128), 0)
            c = lax.broadcasted_iota(jnp.int32, (nrows, 128), 1)
            dist = c + (nrows - 128) - r
            return (dist >= 0) & (dist <= 14) & ((dist & 1) == 0)

        band144 = band(144)

        def qmask(qu, h):
            return pltpu.bitcast(jnp.where(lane_head == h, qu, jnp.uint32(0)), BF)

        def a_keys(t, g):
            ls = slice(128 * g, 128 * g + 128)
            kc = ka_ref[cur, 64 * t:64 * t + 64, ls]
            kp = ka_ref[prv, T // 2 - 8:T // 2, ls] if t == 0 else ka_ref[cur, 64 * t - 8:64 * t, ls]
            return pltpu.bitcast(jnp.concatenate([kp, kc], axis=0), BF)

        a_group_s = {}

        def a_qk(u):
            t, g, h = u
            qu = qa_ref[64 * t:64 * t + 64, 128 * g:128 * g + 128]
            if cfg["a_group_qk"]:
                if h == 0:
                    qs = pltpu.bitcast(jnp.concatenate(
                        [jnp.where(lane_head == hh, qu, jnp.uint32(0)) for hh in range(4)], axis=0), BF)
                    a_group_s[(t, g)] = _dot_nt(a_keys(t, g), qs)
                return a_group_s[(t, g)][:, 128 * h:128 * h + 128]
            return _dot_nt(a_keys(t, g), qmask(qu, h))

        def a_sm(u, s):
            t, g, h = u
            if t == 0:
                s = jnp.concatenate([s[0:16] + bias, s[16:]], axis=0)
            s = jnp.where(band144, s, NEG)
            m = jnp.max(s, axis=0, keepdims=True)
            p = jnp.exp2(s - m)
            l = jnp.sum(p, axis=0, keepdims=True)
            p = jnp.concatenate([jnp.zeros((112, 128), F32), p], axis=0)
            return p.astype(BF), l

        def a_pv(u, pt, l):
            t, g, h = u
            f2 = (128 * g + 32 * h) // 2
            vc = vta_ref[cur, f2:f2 + 16, 128 * t:128 * t + 128]
            vp = (vta_ref[prv, f2:f2 + 16, T - 128:T] if t == 0
                  else vta_ref[cur, f2:f2 + 16, 128 * t - 128:128 * t])
            v = jnp.concatenate([vp, vc], axis=1)
            o = _dot(pltpu.bitcast(v, BF), pt)
            ota_ref[f2:f2 + 16, 128 * t:128 * t + 128] = pltpu.bitcast((o * (1.0 / l)).astype(BF), U32)

        def b_tiles(t):
            return [(prv, 0), (prv, 1), (cur, 0)] if t == 0 else [(prv, 1), (cur, 0), (cur, 1)]

        def b_qk(u):
            t, g, h = u
            ls = slice(128 * g, 128 * g + 128)
            k = jnp.concatenate([kb_ref[sl, 64 * r:64 * r + 64, ls] for sl, r in b_tiles(t)], axis=0)
            return _dot_nt(pltpu.bitcast(k, BF), qmask(qb_ref[64 * t:64 * t + 64, ls], h))

        def red8(x):
            return jnp.max(x.reshape(x.shape[0] // 8, 8, 128), axis=0)

        def b_sm(u, s):
            t = u[0]
            c = jnp.where(upper, s[0:128] + bias, s[256:384])
            mid = s[128:256]
            if t == 0:
                m8 = jnp.maximum(red8(c), red8(mid) + bias)
            else:
                m8 = jnp.maximum(red8(c), red8(mid))
            m = jnp.max(m8, axis=0, keepdims=True)
            pc = jnp.exp2(c - m)
            pm = jnp.exp2(mid - (m - bias if t == 0 else m))
            l = jnp.sum(jnp.concatenate([pc, pm], axis=0), axis=0, keepdims=True)
            pt = jnp.concatenate([jnp.where(upper, pc, 0.0), pm, jnp.where(upper, 0.0, pc)], axis=0)
            return pt.astype(BF), l

        def b_pv(u, pt, l):
            t, g, h = u
            f2 = (128 * g + 32 * h) // 2
            v = jnp.concatenate(
                [vtb_ref[sl, f2:f2 + 16, 128 * r:128 * r + 128] for sl, r in b_tiles(t)], axis=1)
            o = _dot(pltpu.bitcast(v, BF), pt)
            otb_ref[f2:f2 + 16, 128 * t:128 * t + 128] = pltpu.bitcast((o * (1.0 / l)).astype(BF), U32)

        def outp(br, c0, cw):
            ot_ref, wo_ref = (ota_ref, woa_ref) if br == 0 else (otb_ref, wob_ref)
            need("woa" if br == 0 else "wob")
            need_obuf(br)
            r = lax.dot_general(pltpu.bitcast(ot_ref[...], BF), wo_ref[:, c0:c0 + cw], _TN_DIMS,
                                preferred_element_type=F32)
            (oa_buf, ob_buf)[br][cur, :, c0:c0 + cw] = r.astype(BF)
            if br == 1:
                ocopy(1 + c0 // OB, i, cur).start()
            elif c0 + cw == D:
                ocopy(0, i, cur).start()

        def pipeline(units, qk, sm, pv, skew, fillers, tail):
            n_u = len(units)
            s1 = skew // 2
            ss, ps = {}, {}
            nf = len(fillers)
            fi = 0
            for n in range(n_u + skew):
                if n < n_u:
                    ss[n] = qk(units[n])
                if 0 <= n - s1 < n_u:
                    ps[n - s1] = sm(units[n - s1], ss.pop(n - s1))
                if 0 <= n - skew < n_u:
                    pv(units[n - skew], *ps.pop(n - skew))
                while fi < nf and (fi + 1) * n_u <= (n + 1) * nf:
                    fillers[fi]()
                    fi += 1
                if n >= n_u and tail:
                    tail.pop(0)()
            while fi < nf:
                fillers[fi]()
                fi += 1
            while tail:
                tail.pop(0)()

        units = [(t, g, h) for t in range(NT) for g in range(D // 128) for h in range(4)]

        def proj_list(br, cw):
            return [(lambda c=c, part=part: proj(br, part, c, cw))
                    for c0 in range(0, D, max(cw, PC)) for part in range(3)
                    for c in range(c0, c0 + max(cw, PC), cw)]

        pa = proj_list(0, cfg["pa_chunk"])
        pb = proj_list(1, cfg["pb_chunk"])
        for f in pa:
            f()
        if not cfg["fill_a"]:
            for f in pb:
                f()
            pb = []
        pipeline(units, a_qk, a_sm, a_pv, cfg["skew_a"], pb, [])
        oc = cfg["ochunk"]
        oa = [(lambda c=c: outp(0, c, oc)) for c in range(0, D, oc)]
        if cfg["fill_b"]:
            tk = cfg["tail_keep"]
            fill, tail = oa[:len(oa) - tk], oa[len(oa) - tk:]
        else:
            for f in oa:
                f()
            fill, tail = [], []
        pipeline(units, b_qk, b_sm, b_pv, cfg["skew_b"], fill, tail)
        for c in range(0, D, cfg["obchunk"]):
            outp(1, c, cfg["obchunk"])

    step()

    @pl.when(last)
    def _():
        for piece in range(1 + n_ob):
            ocopy(piece, i, cur).wait()

        @pl.when(i >= 1)
        def _():
            for piece in range(1 + n_ob):
                ocopy(piece, i - 1, prv).wait()


def _flags():
    f = {}
    if CFG["resched"]:
        f["XLA_TPU_RESCHEDULE_DMA_DONES"] = True
    if CFG.get("lp"):
        f["XLA_TPU_FORCE_LP_LLO_SCHEDULER"] = True
    if CFG.get("even"):
        f["XLA_TPU_EVENLY_DISTRIBUTE_CRITICAL_NODES"] = True
    return f or None


@jax.jit
def pallas_concat_heads__sliding_local_dilated__sliding_block__prompt_kernel(
    A_x, A_wqkv, A_wo, B_x, B_wqkv, B_wo,
):
    xa = A_x.reshape(S, D)
    xb = B_x.reshape(S, D)
    hbm = pl.BlockSpec(memory_space=pl.ANY)
    n_sem = 2 * 3 * (D // CFG["pchunk"]) + 2
    out = pl.pallas_call(
        _kernel,
        grid=(CFG.get("nsteps", S // T),),
        in_specs=[hbm] * 6,
        out_specs=hbm,
        out_shape=jax.ShapeDtypeStruct((S, 2 * D), BF),
        scratch_shapes=[
            pltpu.VMEM((2, T, D), BF), pltpu.VMEM((2, T, D), BF),
            pltpu.VMEM((2, T, D), BF), pltpu.VMEM((2, T, D), BF),
            pltpu.VMEM((D, 3 * D), BF), pltpu.VMEM((D, 3 * D), BF),
            pltpu.VMEM((D, D), BF), pltpu.VMEM((D, D), BF),
            pltpu.VMEM((T // 2, D), U32), pltpu.VMEM((2, T // 2, D), U32),
            pltpu.VMEM((2, D // 2, T), U32), pltpu.VMEM((D // 2, T), U32),
            pltpu.VMEM((T // 2, D), U32), pltpu.VMEM((2, T // 2, D), U32),
            pltpu.VMEM((2, D // 2, T), U32), pltpu.VMEM((D // 2, T), U32),
            pltpu.SemaphoreType.DMA((n_sem,)),
            pltpu.SemaphoreType.DMA((2, 2)),
            pltpu.SemaphoreType.DMA((2, 1 + D // CFG["obchunk"])),
        ],
        compiler_params=pltpu.CompilerParams(
            dimension_semantics=("arbitrary",),
            vmem_limit_bytes=100 * 1024 * 1024,
            flags=_flags(),
        ),
        name="fused_attn",
    )(xa, A_wqkv, A_wo, xb, B_wqkv, B_wo)
    return out.reshape(1, S, 2 * D)
```

```python
import jax
import jax.numpy as jnp
import numpy as np
from jax import lax
from jax.experimental import pallas as pl
from jax.experimental.pallas import tpu as pltpu

S, D, DH = 2048, 1024, 32
T = 256
NT = T // 128
NG = D // 128
PC = 512
FC = 128
OB = 512
WINDOW = 3
SKEW_A, SKEW_B = 6, 14
NEG = -1e30
BF, F32, U32 = jnp.bfloat16, jnp.float32, jnp.uint32
QSCALE = float(DH ** -0.5 * np.log2(np.e))


def _dot(a, b):
    return jnp.dot(a, b, preferred_element_type=F32)


def _dot_nt(a, b):
    return lax.dot_general(a, b, (((1,), (1,)), ((), ())), preferred_element_type=F32)


def _bf(x):
    return pltpu.bitcast(x, BF)


def _u32(x):
    return pltpu.bitcast(x.astype(BF), U32)


def _iota(shape, dim):
    return lax.broadcasted_iota(jnp.int32, shape, dim)


def _pipeline(units, qk, sm, pv, skew, fillers, tail):
    n_u = len(units)
    ss, ps, at = {}, {}, {}
    for fl, lo, hi in fillers:
        for j, f in enumerate(fl):
            at.setdefault(lo + ((j + 1) * (hi - lo) - 1) // len(fl), []).append(f)
    for n in range(n_u + skew):
        if n < n_u:
            ss[n] = qk(units[n])
        if 0 <= n - skew // 2 < n_u:
            ps[n - skew // 2] = sm(units[n - skew // 2], ss.pop(n - skew // 2))
        if 0 <= n - skew < n_u:
            pv(units[n - skew], *ps.pop(n - skew))
        for f in at.pop(n, []):
            f()
        if n >= n_u and tail:
            tail.pop(0)()


def _kernel(xa_hbm, wa_hbm, woa_hbm, xb_hbm, wb_hbm, wob_hbm, o_hbm,
            xa_buf, xb_buf, oa_buf, ob_buf, wa_ref, wb_ref, woa_ref, wob_ref,
            qa_ref, ka_ref, vta_ref, vca_ref, ona_ref, qb_ref, kb_ref, vtb_ref, onb_ref,
            wsems, xsems, osems):
    i = pl.program_id(0)
    first = i == 0
    last = i == pl.num_programs(0) - 1
    cur = i % 2
    prv = 1 - cur
    bias = jnp.where(first, jnp.float32(NEG), jnp.float32(0.0))

    wcopies, widx = [], {}
    for br, (w_hbm, w_ref) in enumerate(((wa_hbm, wa_ref), (wb_hbm, wb_ref))):
        for c in range(0, D, PC):
            for part in range(3):
                widx[br, part, c] = len(wcopies)
                cols = slice(part * D + c, part * D + c + PC)
                wcopies.append((w_hbm.at[:, cols], w_ref.at[:, cols]))
    for key, pair in (("woa", (woa_hbm, woa_ref)), ("wob", (wob_hbm, wob_ref)),
                      ("xb0", (xb_hbm.at[0:T, :], xb_buf.at[0]))):
        widx[key] = len(wcopies)
        wcopies.append(pair)

    def wcopy(j):
        return pltpu.make_async_copy(*wcopies[j], wsems.at[j])

    def xcopy(br, step, slot):
        src = (xa_hbm, xb_hbm)[br].at[pl.ds(pl.multiple_of(step * T, T), T), :]
        return pltpu.make_async_copy(src, (xa_buf, xb_buf)[br].at[slot], xsems.at[br, slot])

    def ocopy(piece, step, slot):
        rows = pl.ds(pl.multiple_of(step * T, T), T)
        if piece == 0:
            return pltpu.make_async_copy(oa_buf.at[slot], o_hbm.at[rows, 0:D], osems.at[slot, 0])
        c0 = (piece - 1) * OB
        return pltpu.make_async_copy(ob_buf.at[slot, :, c0:c0 + OB],
                                     o_hbm.at[rows, D + c0:D + c0 + OB], osems.at[slot, piece])

    queue = ["xa0"] + list(range(widx["xb0"]))
    queue.insert(7, widx["xb0"])
    queue.insert(len(queue) - 1, "x1")
    n_started, n_done = [0], [0]

    def start_upto(n):
        lo, hi = n_started[0], min(n, len(queue))
        if hi > lo:
            @pl.when(first)
            def _():
                for item in queue[lo:hi]:
                    if item == "x1":
                        @pl.when(jnp.logical_not(last))
                        def _():
                            xcopy(0, 1, 1).start()
                            xcopy(1, 1, 1).start()
                    elif item == "xa0":
                        xcopy(0, 0, 0).start()
                    else:
                        wcopy(item).start()
            n_started[0] = hi

    def need(item):
        while n_done[0] <= queue.index(item):
            head = queue[n_done[0]]
            if head == "xa0":
                xcopy(0, i, cur).wait()
            elif head != "x1":
                @pl.when(first)
                def _(head=head):
                    wcopy(head).wait()
            n_done[0] += 1
            start_upto(n_done[0] + WINDOW)

    once = set()

    def need_x(br):
        if br == 0:
            need("xa0")
        elif "xb" not in once:
            once.add("xb")
            need(widx["xb0"])

            @pl.when(jnp.logical_not(first))
            def _():
                xcopy(1, i, cur).wait()

    def need_obuf(br):
        if ("o", br) not in once:
            once.add(("o", br))

            @pl.when(i >= 2)
            def _():
                for piece in ([0] if br == 0 else range(1, 1 + D // OB)):
                    ocopy(piece, i - 2, cur).wait()

    start_upto(WINDOW)

    @pl.when(jnp.logical_and(jnp.logical_not(first), jnp.logical_not(last)))
    def _():
        xcopy(0, i + 1, prv).start()
        xcopy(1, i + 1, prv).start()

    @pl.when(first)
    def _():
        kb_ref[1] = jnp.zeros(kb_ref.shape[1:], U32)
        vtb_ref[1] = jnp.zeros(vtb_ref.shape[1:], U32)

    row, col = _iota((128, 128), 0), _iota((128, 128), 1)
    older = [row > ((col - DH * h) & 127) for h in range(4)]
    head64 = _iota((64, 128), 1) // DH
    head32 = _iota((32, 128), 1) // DH
    blk16 = _iota((16, 128), 1) // DH
    dist = (_iota((80, 128), 1) & 63) + 16 - _iota((80, 128), 0)
    band = (dist >= 0) & (dist <= 14) & ((dist & 1) == 0)
    low16 = _iota((16, 128), 1) < 64
    even_head = (head32 & 1) == 0

    def proj(br, part, c, cw):
        need_x(br)
        need(widx[br, part, c // PC * PC])
        w_ref = (wa_ref, wb_ref)[br]
        r = _dot((xa_buf, xb_buf)[br][cur], w_ref[:, part * D + c:part * D + c + cw])
        cs = slice(c, c + cw)
        if part == 0:
            (qa_ref, qb_ref)[br][:, cs] = _u32(r * QSCALE)
        elif br == 1 and part == 1:
            kb_ref[cur, :, cs] = _u32(r)
        elif br == 1:
            vtb_ref[cur, c // 2:(c + cw) // 2, :] = pltpu.bitcast(r.astype(BF).T, U32)
        elif part == 1:
            ka_ref[0:8, cs] = jnp.where(first, jnp.uint32(0), ka_ref[T // 2:T // 2 + 8, cs])
            ka_ref[8:8 + T // 2, cs] = _u32(r)
        else:
            vu = _u32(r)
            ext = jnp.concatenate([jnp.where(first, jnp.uint32(0), vca_ref[:, cs]), vu], axis=0)
            for kk in range(T // 64):
                vta_ref[kk, c // 2:(c + cw) // 2, :] = pltpu.bitcast(
                    _bf(ext[32 * kk:32 * kk + 64]).T, U32)
            vca_ref[:, cs] = vu[T // 2 - 32:]

    def proj_list(br, cw):
        return [(lambda c=c, part=part: proj(br, part, c, cw))
                for c0 in range(0, D, PC) for part in range(3) for c in range(c0, c0 + PC, cw)]

    def a_qk(u):
        _, g, kk, pp = u
        ls = slice(128 * g, 128 * g + 128)
        qu = qa_ref[32 * kk:32 * kk + 32, ls]
        heads = [2 * pp + (hs if kk % 2 == 0 else 1 - hs) for hs in range(2)]
        qs = jnp.concatenate([jnp.where(head32 == h, qu, jnp.uint32(0)) for h in heads], axis=0)
        return _dot_nt(_bf(ka_ref[32 * kk:32 * kk + 40, ls]), _bf(qs))

    def a_sm(u, s):
        if u[2] == 0:
            s = jnp.concatenate([s[0:16] + bias, s[16:]], axis=0)
        s = jnp.where(band, s, NEG)
        p = jnp.exp2(s - jnp.max(s, axis=0, keepdims=True))
        l = jnp.sum(p, axis=0, keepdims=True)
        return jnp.concatenate([jnp.zeros((48, 128), F32), p], axis=0).astype(BF), l

    a_out = {}

    def a_pv(u, pt, l):
        t, g, kk, pp = u
        f2 = (128 * g + 64 * pp) // 2
        a_out[kk % 2, pp] = _u32(_dot(_bf(vta_ref[kk, f2:f2 + 32, :]), pt) * (1.0 / l))
        if len(a_out) == 4:
            parts = []
            for p in range(2):
                a0, a1 = a_out.pop((0, p)), a_out.pop((1, p))
                parts.append(jnp.where(low16, a0[0:16], a1[0:16]))
                parts.append(jnp.where(low16, a1[16:32], a0[16:32]))
            zt = pltpu.bitcast(_bf(jnp.concatenate(parts, axis=0)).T, U32)
            top, bot = zt[0:32], zt[32:64]
            ls = slice(128 * g, 128 * g + 128)
            ona_ref[64 * t:64 * t + 32, ls] = jnp.where(even_head, top, bot)
            ona_ref[64 * t + 32:64 * t + 64, ls] = jnp.where(even_head, bot, top)

    def b_tiles(t):
        return [(prv, 0), (prv, 1), (cur, 0)] if t == 0 else [(prv, 1), (cur, 0), (cur, 1)]

    b_grp = {}

    def b_qk(u):
        t, g, h = u
        ls = slice(128 * g, 128 * g + 128)
        kf, km, kl = [kb_ref[sl, 64 * r:64 * r + 64, ls] for sl, r in b_tiles(t)]
        zero = jnp.zeros((16, 128), U32)

        def mm(k, w):
            return _dot(_bf(k), _bf(jnp.concatenate(w, axis=0)))

        if h == 0:
            qu = qb_ref[64 * t:64 * t + 64, ls]
            rot = qu
            for hh in range(1, 4):
                shifted = jnp.concatenate([qu[64 - 16 * hh:], qu[:64 - 16 * hh]], axis=0)
                rot = jnp.where(head64 == hh, shifted, rot)
            qt = pltpu.bitcast(_bf(rot).T, U32)
            rows = [qt[16 * hh:16 * hh + 16] for hh in range(4)]

            def blocks(hh, qbs):
                keep = blk16 == (qbs[0] + hh) % 4
                for qb in qbs[1:]:
                    keep = keep | (blk16 == (qb + hh) % 4)
                return jnp.where(keep, rows[hh], jnp.uint32(0))

            b_grp["rows"] = rows
            b_grp["f0"] = mm(kf[0:16], [blocks(hh, (0,)) for hh in range(4)])
            b_grp["l3"] = mm(kl[48:64], [blocks(hh, (3,)) for hh in range(4)])
            for par in range(2):
                b_grp["f1", par] = mm(kf[16:32], [blocks(hh, (0, 1)) if hh % 2 == par else zero
                                                  for hh in range(4)])
                b_grp["l2", par] = mm(kl[32:48], [blocks(hh, (2, 3)) if hh % 2 == par else zero
                                                  for hh in range(4)])
        s = mm(jnp.concatenate([kf[32:64], km, kl[0:32]], axis=0),
               [b_grp["rows"][hh] if hh == h else zero for hh in range(4)])
        return (jnp.concatenate([b_grp["f0"], b_grp["f1", h % 2], s[0:64]], axis=0), s[64:192],
                jnp.concatenate([s[192:256], b_grp["l2", h % 2], b_grp["l3"]], axis=0))

    def red8(x):
        return jnp.max(x.reshape(x.shape[0] // 8, 8, 128), axis=0)

    def b_sm(u, s):
        t, _, h = u
        s_old, mid, s_new = s
        c = jnp.where(older[h], s_old + bias, s_new)
        m8 = jnp.maximum(red8(c), red8(mid) + bias if t == 0 else red8(mid))
        m = jnp.max(m8, axis=0, keepdims=True)
        pc = jnp.exp2(c - m)
        pm = jnp.exp2(mid - (m - bias if t == 0 else m))
        l = jnp.sum(jnp.concatenate([pc, pm], axis=0), axis=0, keepdims=True)
        pt = jnp.concatenate([jnp.where(older[h], pc, 0.0), pm, jnp.where(older[h], 0.0, pc)], axis=0)
        return pt.astype(BF), l

    b_out = []

    def b_pv(u, pt, l):
        t, g, h = u
        f2 = (128 * g + DH * h) // 2
        v = jnp.concatenate(
            [vtb_ref[sl, f2:f2 + 16, 128 * r:128 * r + 128] for sl, r in b_tiles(t)], axis=1)
        b_out.append(_u32(_dot(_bf(v), pt) * (1.0 / l)))
        if len(b_out) == 4:
            zt = pltpu.bitcast(_bf(jnp.concatenate(b_out, axis=0)).T, U32)
            del b_out[:]
            nat = zt
            for hh in range(1, 4):
                back = jnp.concatenate([zt[16 * hh:], zt[:16 * hh]], axis=0)
                nat = jnp.where(head64 == hh, back, nat)
            onb_ref[64 * t:64 * t + 64, 128 * g:128 * g + 128] = nat

    def outp(br, c, cw):
        need(widx["woa" if br == 0 else "wob"])
        need_obuf(br)
        r = _dot(_bf((ona_ref, onb_ref)[br][...]), (woa_ref, wob_ref)[br][:, c:c + cw])
        (oa_buf, ob_buf)[br][cur, :, c:c + cw] = r.astype(BF)
        if br == 1:
            ocopy(1 + c // OB, i, cur).start()
        elif c + cw == D:
            ocopy(0, i, cur).start()

    units_a = [(t, g, 2 * t + uu, pp) for g in range(NG) for t in range(NT)
               for uu in range(2) for pp in range(2)]
    units_b = [(t, g, h) for g in range(NG) for t in range(NT) for h in range(4)]
    half = len(units_b) // 2
    pb = proj_list(1, FC)
    oa = [(lambda c=c: outp(0, c, FC)) for c in range(0, D, FC)]

    for f in proj_list(0, PC):
        f()
    _pipeline(units_a, a_qk, a_sm, a_pv, SKEW_A, [(pb[:len(pb) // 2], 0, len(units_a))], [])
    _pipeline(units_b, b_qk, b_sm, b_pv, SKEW_B,
              [(pb[len(pb) // 2:], 0, half - 2), (oa[:-1], half, len(units_b))], oa[-1:])
    for c in range(0, D, OB):
        outp(1, c, OB)

    @pl.when(last)
    def _():
        for piece in range(1 + D // OB):
            ocopy(piece, i, cur).wait()

        @pl.when(i >= 1)
        def _():
            for piece in range(1 + D // OB):
                ocopy(piece, i - 1, prv).wait()


@jax.jit
def pallas_concat_heads__sliding_local_dilated__sliding_block__prompt_kernel(
    A_x: jax.Array,
    A_wqkv: jax.Array,
    A_wo: jax.Array,
    B_x: jax.Array,
    B_wqkv: jax.Array,
    B_wo: jax.Array,
):
    hbm = pl.BlockSpec(memory_space=pl.ANY)
    out = pl.pallas_call(
        _kernel,
        grid=(S // T,),
        in_specs=[hbm] * 6,
        out_specs=hbm,
        out_shape=jax.ShapeDtypeStruct((S, 2 * D), BF),
        scratch_shapes=[
            pltpu.VMEM((2, T, D), BF), pltpu.VMEM((2, T, D), BF),
            pltpu.VMEM((2, T, D), BF), pltpu.VMEM((2, T, D), BF),
            pltpu.VMEM((D, 3 * D), BF), pltpu.VMEM((D, 3 * D), BF),
            pltpu.VMEM((D, D), BF), pltpu.VMEM((D, D), BF),
            pltpu.VMEM((T // 2, D), U32),
            pltpu.VMEM((8 + T // 2, D), U32),
            pltpu.VMEM((T // 64, D // 2, 128), U32),
            pltpu.VMEM((32, D), U32),
            pltpu.VMEM((T // 2, D), U32),
            pltpu.VMEM((T // 2, D), U32),
            pltpu.VMEM((2, T // 2, D), U32),
            pltpu.VMEM((2, D // 2, T), U32),
            pltpu.VMEM((T // 2, D), U32),
            pltpu.SemaphoreType.DMA((2 * 3 * (D // PC) + 3,)),
            pltpu.SemaphoreType.DMA((2, 2)),
            pltpu.SemaphoreType.DMA((2, 1 + D // OB)),
        ],
        compiler_params=pltpu.CompilerParams(
            dimension_semantics=("arbitrary",),
            vmem_limit_bytes=100 * 1024 * 1024,
            flags={"XLA_TPU_RESCHEDULE_DMA_DONES": True},
        ),
        name="fused_attn",
    )(A_x.reshape(S, D), A_wqkv, A_wo, B_x.reshape(S, D), B_wqkv, B_wo)
    return out.reshape(1, S, 2 * D)
```
